```python
import os as _os
_os.environ.setdefault("JAX_PLATFORMS", "cpu")
import jax
import jax.numpy as jnp

def _softmax(x, axis=-1):
    return jax.nn.softmax(x, axis=axis)
def _gelu(x):
    return jax.nn.gelu(x, approximate=True)
def _silu(x):
    return jax.nn.silu(x)
def _sigmoid(x):
    return jax.nn.sigmoid(x)
def _layernorm(x, axis=-1, eps=1e-5):
    m = jnp.mean(x, axis=axis, keepdims=True)
    v = jnp.var(x, axis=axis, keepdims=True)
    return (x - m) / jnp.sqrt(v + eps)
def _scatter_add(tgt, idx, src, axis=0):
    return tgt.at[idx].add(src)
def _segment_sum(src, seg, n):
    return jax.ops.segment_sum(src, seg, n)
class _Rng:
    def __init__(self, key):
        self._k = key
    def _next(self):
        self._k, sub = jax.random.split(self._k)
        return sub
    def normal(self, shape):
        return jax.random.normal(self._next(), shape, dtype=jnp.bfloat16)
    def randint(self, lo, hi, shape):
        return jax.random.randint(self._next(), shape, lo, hi, dtype=jnp.int32)
    def uniform(self, shape, lo=0.0, hi=1.0):
        return jax.random.uniform(self._next(), shape, jnp.bfloat16, lo, hi)
    def permutation(self, n):
        return jax.random.permutation(self._next(), n)


kernel_name = 'concat_heads__sliding_local_dilated__sliding_block__prompt'

def setup_inputs():
    _rng = _Rng(jax.random.key(int.from_bytes(__import__("os").urandom(4), "little")))
    _w = (lambda a: (lambda t: t.astype(jnp.bfloat16) if jnp.issubdtype(t.dtype, jnp.floating) else t)(jnp.asarray(a)))
    def _A_setup():
        B, S, D = 1, 2048, 1024
        return {
            "x": _w((lambda *s: _rng.normal(s) * 0.2)(B, S, D)),
            "wqkv": _w((lambda *s: _rng.normal(s) * 0.2)(D, 3 * D)),
            "wo": _w((lambda *s: _rng.normal(s) * 0.05)(D, D)),
        }
    _A_in = _A_setup()

    def _B_setup():
        B, S, D = 1, 2048, 1024
        return {
            "x": _w((lambda *s: _rng.normal(s) * 0.2)(B, S, D)),
            "wqkv": _w((lambda *s: _rng.normal(s) * 0.2)(D, 3 * D)),
            "wo": _w((lambda *s: _rng.normal(s) * 0.05)(D, D)),
        }
    _B_in = _B_setup()

    return {
        "A_x": _A_in["x"],
        "A_wqkv": _A_in["wqkv"],
        "A_wo": _A_in["wo"],
        "B_x": _B_in["x"],
        "B_wqkv": _B_in["wqkv"],
        "B_wo": _B_in["wo"],
    }

def reference(A_x, A_wqkv, A_wo, B_x, B_wqkv, B_wo):
    def _A_ref(x, wqkv, wo):
        B, S, D = x.shape
        H = 32; Dh = D // H
        W, dil = 8, 2
        qkv = (lambda x, *d: x.transpose(*d))((x @ wqkv).reshape(B, S, 3, H, Dh), 2, 0, 3, 1, 4)
        q, k, v = qkv[0], qkv[1], qkv[2]
        scale = Dh ** -0.5
        pos = jnp.arange(S)
        off = jnp.arange(W) * dil
        idx = pos[:, None] - off[None, :]
        mask = idx >= 0
        idx_c = jnp.where(mask, idx, 0).reshape(-1)
        kg = k[:, :, idx_c, :].reshape(B, H, S, W, Dh)
        vg = v[:, :, idx_c, :].reshape(B, H, S, W, Dh)
        logits = jnp.einsum("bhsd,bhswd->bhsw", q, kg) * scale
        logits = jnp.where(mask[None, None, :, :], logits, -1e9)
        attn = _softmax(logits, axis=-1)
        o = jnp.einsum("bhsw,bhswd->bhsd", attn, vg)
        return (lambda x, *d: x.transpose(*d))(o, 0, 2, 1, 3).reshape(B, S, D) @ wo

    def _B_ref(x, wqkv, wo):
        B, S, D = x.shape
        H = 32; Dh = D // H; W = 256
        qkv = (lambda x, *d: x.transpose(*d))((x @ wqkv).reshape(B, S, 3, H, Dh), 2, 0, 3, 1, 4)
        q, k, v = qkv[0], qkv[1], qkv[2]
        scores = jnp.einsum("bhqd,bhkd->bhqk", q, k) * (Dh ** -0.5)
        idx = jnp.arange(S)
        mask = (idx[:, None] - idx[None, :] >= 0) & (idx[:, None] - idx[None, :] < W)
        scores = jnp.where(mask[None, None], scores, -1e9)
        p = _softmax(scores, axis=-1)
        o = jnp.einsum("bhqk,bhkd->bhqd", p, v)
        return (lambda x, *d: x.transpose(*d))(o, 0, 2, 1, 3).reshape(B, S, D) @ wo

    a = _A_ref(A_x, A_wqkv, A_wo)
    b = _B_ref(B_x, B_wqkv, B_wo)
    return jnp.concatenate([a, b], axis=-1)
```

```python
import contextlib
import functools
import numpy as np
import jax
import jax.numpy as jnp
from jax import lax
from jax.experimental import pallas as pl
from jax.experimental.pallas import tpu as pltpu

S, D, H, DH = 2048, 1024, 32, 32
T = 256
NQB = T // 128
NSTEP = S // T
LOG2E = 1.4426950408889634
SCALE = DH ** -0.5
NEG = -1e30
bf = jnp.bfloat16
f32 = jnp.float32
u32 = jnp.uint32

NT = (((1,), (1,)), ((), ()))

LAG_B = 1
LAG_A = 2
SKIP_B = 1
SKIP_A = 0
END_B = 4
END_A = 0
SCOPES = 0
KA0 = 1
PW = 256
PSTART = 2
PTAIL = 2
MERGE_B = 1
EOFF_B = 0
EOFF_A = 0
PVFRAC = {"B": 0 / 100, "A": 0 / 100}
MERGE_A = 1
FLAGS = {}


def scope(n):
    on = SCOPES == 1 or (SCOPES >= 2 and n in ("wait0", "xwait", "tail"))
    return jax.named_scope(n) if on else contextlib.nullcontext()


b2u = lambda x: pltpu.bitcast(x, u32)
u2b = lambda x: pltpu.bitcast(x, bf)

KR = 2 * (T // 2)
PB0 = KR
LB0 = PB0 + 192
XB0 = LB0 + 32
STROWS = XB0 + T // 2


class Filler:
    def __init__(self):
        self.items = []

    def add(self, fn):
        self.items.append(fn)

    def flush(self, n=None):
        n = len(self.items) if n is None else min(n, len(self.items))
        for _ in range(n):
            self.items.pop(0)()

    def spread(self, nchunks, skip, end, keep=0):
        n = len(self.items) - keep
        act = max(1, nchunks - skip - end)
        done = 0
        res = []
        for j in range(nchunks):
            due = 0 if j < skip else min(n, -(-(j - skip + 1) * n // act))
            res.append(due - done)
            done = due
        return res


def _body(first, step, z, z1, xa, xb, wa, wb, woa, wob, out,
          qa, qb_, stA, stB, ka, pa, vta, vtb, ota, otb, ona, s_sc, biasb, biasa, biasm, biasa4, wait):
    def scope(n):
        on = SCOPES == 1 or (SCOPES == 3 and first)
        return jax.named_scope(n) if on else contextlib.nullcontext()

    if first:
        cur, prv = 0, None
        zk = z
        zkp = None
    else:
        cur = lax.rem(step, 2)
        prv = 1 - cur
        zk = pl.multiple_of(z + cur * (T // 2), 8)
        zkp = pl.multiple_of(z + prv * (T // 2), 8)
    lane32 = lax.broadcasted_iota(jnp.int32, (64, 128), 1)
    hmask = [(lane32 >= 32 * h) & (lane32 < 32 * h + 32) for h in range(4)]
    fill = Filler()

    def ds8(zz, off, n):
        if isinstance(zz, int):
            return slice(zz + off, zz + off + n)
        return pl.ds(pl.multiple_of(zz + off, 8), n)
    zero = jnp.uint32(0)

    def proj(xv, w_ref, c0, n=D):
        return jnp.dot(xv, w_ref[:, c0:c0 + n], preferred_element_type=f32)

    def store_k(st, k, c0=0):
        ku = b2u(k.astype(bf))
        n = k.shape[1]
        if first:
            st[0:T // 2, c0:c0 + n] = ku
        else:
            st[pl.ds(pl.multiple_of(cur * (T // 2), 8), T // 2), c0:c0 + n] = ku

    def store_vt(vt, v):
        vT = b2u(v.astype(bf).T)
        if first:
            vt[0] = vT
        else:
            vt[cur] = vT

    def anchored(st, row0, nchunk):
        sp = fill.spread(nchunk, 0, 1)
        cs = []
        for j in range(nchunk):
            fill.flush(sp[j])
            cs.append(u2b(st[pl.ds(pl.multiple_of(z + row0 + 8 * j, 8), 8), :]))
        fill.flush()
        return jnp.concatenate(cs, axis=0)

    class Att:
        def __init__(self, br):
            self.br = br
            isB = br == "B"
            self.hist = 256 if isB else 16
            self.q = qb_ if isB else qa
            self.st = stB if isB else ka
            self.pst = stB if isB else pa
            self.pz = z if isB else 0
            self.p0 = PB0 if isB else 0
            self.l0 = LB0 if isB else 192
            self.jobs = {}
            self.vt = vtb if isB else vta
            self.ot = otb if isB else ota
            self.on = (stA, XB0) if isB else (ona, 0)
            self.lag = LAG_B if isB else LAG_A
            self.eoff = EOFF_B if isB else EOFF_A
            self.nsb = self.lag - self.eoff + 1
            self.pvfrac = 0.0
            self.skip = SKIP_B if isB else SKIP_A
            self.end = END_B if isB else END_A
            self.units = [(g, qb) for g in range(8) for qb in range(NQB)]
            self.ms = {}
            self.ls = {}

        def nk(self, qb):
            if first:
                return min(self.hist, 128 * qb) + 128
            return self.hist + 128

        def kchunk(self, g, qb, j):
            nk = self.nk(qb)
            r = 128 * qb + 128 - nk + 16 * j
            if r < 0:
                base, rr = zkp, (r + T) // 2
            else:
                base, rr = zk, r // 2
            return self.st[pl.ds(pl.multiple_of(base + rr, 8), 8), 128 * g:128 * g + 128]

        def qtile(self, u):
            g, qb = self.units[u]
            return self.q[64 * qb:64 * qb + 64, 128 * g:128 * g + 128]

        def merged(self, u):
            g, qb = self.units[u]
            return self.nk(qb) == self.hist + 128 and (MERGE_B if self.br == "B" else MERGE_A)

        def kloads(self, u, early=()):
            g, qb = self.units[u]
            nch = self.nk(qb) // 16
            ks = [None] * nch
            for j in early:
                ks[j] = self.kchunk(g, qb, j)
            rest = [j for j in range(nch) if j not in early]
            keep = int(len(fill.items) * self.pvfrac)
            sp = fill.spread(len(rest), min(self.skip, len(rest) // 3), min(self.end, len(rest) // 4), keep)
            for i, j in enumerate(rest):
                fill.flush(sp[i])
                ks[j] = self.kchunk(g, qb, j)
            fill.flush(len(fill.items) - keep)
            return ks

        def put(self, sb, h, parts):
            m = None
            for r0, p in parts:
                mm = jnp.max(p, axis=0, keepdims=True)
                m = mm if m is None else jnp.maximum(m, mm)
                sb[h, r0:r0 + p.shape[0], :] = p
            return m

        def qk(self, u):
            if self.merged(u):
                return (self.qk_b2 if self.br == "B" else self.qk_a4)(u)
            g, qb = self.units[u]
            nk = self.nk(qb)
            qi = self.qtile(u)
            qw = jnp.concatenate([u2b(jnp.where(hmask[h], qi, zero)) for h in range(4)], axis=0)
            ks = self.kloads(u)
            st = lax.dot_general(u2b(jnp.concatenate(ks, axis=0)), qw, NT, preferred_element_type=f32)
            sb = s_sc[u % self.nsb]
            ms = []
            for h in range(4):
                s = st[:, 128 * h:128 * h + 128]
                parts = []
                if self.br == "B":
                    nt = nk // 128
                    for t in range(nt):
                        p = s[128 * t:128 * t + 128]
                        if t == nt - 1:
                            p = p + biasb[1]
                        elif t == 0 and nt == 3:
                            p = p + biasb[0]
                        parts.append((128 * t, p))
                else:
                    parts.append((0, s + biasa[144 - nk:144, :]))
                ms.append(self.put(sb, h, parts))
            self.ms[u] = ms

        def qk_b2(self, u):
            qi = self.qtile(u)
            qm = [jnp.where(hmask[h], qi, zero) for h in range(4)]
            qr = pltpu.roll(qi[32:64], 32, 1)
            qx = [jnp.concatenate([qm[h][0:32], jnp.where(hmask[(h + 1) % 4][0:32], qr, zero)], axis=0) for h in range(4)]
            ks = self.kloads(u, early=(20, 21, 22, 23, 0, 1, 2, 3))
            ka = jnp.concatenate(ks[0:4], axis=0)
            kb = pltpu.roll(jnp.concatenate(ks[20:24], axis=0), 32, 1)
            even = (lane32[0:32] & 32) == 0
            l1 = u2b(jnp.where(even, ka, kb))
            l2 = u2b(jnp.where(even, kb, ka))
            s1 = lax.dot_general(l1, u2b(jnp.concatenate([qx[0], qx[2]], axis=0)), NT, preferred_element_type=f32)
            s2 = lax.dot_general(l2, u2b(jnp.concatenate([qx[1], qx[3]], axis=0)), NT, preferred_element_type=f32)
            main = u2b(jnp.concatenate(ks[4:20], axis=0))
            st = lax.dot_general(main, u2b(jnp.concatenate(qm, axis=0)), NT, preferred_element_type=f32)
            sb = s_sc[u % self.nsb]
            ms = []
            for h in range(4):
                s = st[:, 128 * h:128 * h + 128]
                sm = (s1, s2)[h % 2][:, 128 * (h // 2):128 * (h // 2) + 128]
                parts = [(0, sm + biasm[...]), (64, s[0:64] + biasb[0, 64:128, :]), (128, s[64:192]),
                         (256, s[192:256] + biasb[1, 0:64, :])]
                ms.append(self.put(sb, h, parts))
            self.ms[u] = ms

        def qk_a4(self, u):
            qi = self.qtile(u)
            qr = [qi[0:16]] + [pltpu.roll(qi[16 * m:16 * m + 16], 32 * m, 1) for m in (1, 2, 3)]
            ks = self.kloads(u)
            kr = []
            for m in range(4):
                w = jnp.concatenate(ks[2 * m:2 * m + 3], axis=0)
                kr.append(w if m == 0 else pltpu.roll(w, 32 * m, 1))
            grp = lane32[0:24] >> 5
            sb = s_sc[u % self.nsb]
            ms = []
            for h in range(4):
                rel = (grp - h) & 3
                lhs = jnp.where(rel == 0, kr[0], jnp.where(rel == 1, kr[1], jnp.where(rel == 2, kr[2], kr[3])))
                w = jnp.concatenate([jnp.where(hmask[(h + m) % 4][0:16], qr[m], zero) for m in range(4)], axis=0)
                s = lax.dot_general(u2b(lhs), u2b(w), NT, preferred_element_type=f32)
                ms.append(self.put(sb, h, [(0, s + biasa4[...])]))
            self.ms[u] = ms

        def nexp(self, u):
            g, qb = self.units[u]
            if self.merged(u):
                return 20 if self.br == "B" else 3
            return self.nk(qb) // 16

        def queue_exp(self, u):
            nch = self.nexp(u)
            ls = [None] * 4
            self.ls[u] = ls
            ms = self.ms[u]
            sb = s_sc[u % self.nsb]
            lane0 = 512 * (u % 2)

            def mk(h, r):
                def fn():
                    s = sb[h + z1, 16 * r:16 * r + 16, :]
                    p = jnp.exp2(s - ms[h])
                    acc = p[0:8] + p[8:16]
                    ls[h] = acc if ls[h] is None else ls[h] + acc
                    self.pst[ds8(self.pz, self.p0 + 8 * r, 8), lane0 + 128 * h:lane0 + 128 * h + 128] = b2u(p.astype(bf))
                    if (r % 8 == 7 or r == nch - 1) and self.br == "B":
                        self.pst[ds8(self.pz, self.l0 + 8 * h, 8), lane0 + 128 * h:lane0 + 128 * h + 128] = pltpu.bitcast(ls[h], u32)
                return fn
            for h in range(4):
                for r in range(nch):
                    fill.add(mk(h, r))

        def pv(self, u):
            g, qb = self.units[u]
            nk = self.nk(qb)
            lane0 = 512 * (u % 2)
            nt = -(-nk // 128)
            mg = self.merged(u)
            for h in range(4):
                r0 = 64 * g + 16 * h
                tiles = []
                for t in range(nt):
                    kt = qb - (nt - 1 - t)
                    if kt < 0:
                        tiles.append(self.vt[prv, r0:r0 + 16, 128 * (kt + NQB):128 * (kt + NQB) + 128])
                    elif first:
                        tiles.append(self.vt[0, r0:r0 + 16, 128 * kt:128 * kt + 128])
                    else:
                        tiles.append(self.vt[cur, r0:r0 + 16, 128 * kt:128 * kt + 128])
                vt = u2b(jnp.concatenate(tiles, axis=1))
                n = self.nexp(u) * 8
                fill.flush(-(-len(fill.items) // (4 - h)) if h else len(fill.items) // 5)
                p = self.pst[ds8(self.pz, self.p0, n), lane0 + 128 * h:lane0 + 128 * h + 128]
                if mg and self.br == "B":
                    lo = lane32[0:32] < 64
                    p = jnp.concatenate([jnp.where(lo, p[0:32], zero), p[32:160], jnp.where(lo, zero, p[0:32])], axis=0)
                elif mg:
                    gm = [hmask[m][0:8] for m in range(4)]
                    p0, p1, p2 = p[0:8], p[8:16], p[16:24]
                    lo2 = [lane32[0:8] < 32 * (m + 1) for m in range(4)]
                    rows = [jnp.where(gm[0], p0, zero), jnp.where(gm[0], p1, zero)]
                    for m in range(3):
                        rows.append(jnp.where(gm[m], p2, jnp.where(gm[m + 1], p0, zero)))
                        rows.append(jnp.where(gm[m + 1], p1, zero))
                    rows.append(jnp.where(gm[3], p2, zero))
                    p = jnp.concatenate(rows, axis=0)
                if nk % 128:
                    p = jnp.concatenate([jnp.zeros(((128 * nt - nk) // 2, 128), u32), p], axis=0)
                ot = jnp.dot(vt, u2b(p), preferred_element_type=f32)
                l = jnp.sum(self.ls[u][h], axis=0, keepdims=True)
                self.ot[r0:r0 + 16, 128 * qb:128 * qb + 128] = b2u((ot * (1.0 / l)).astype(bf))
            fill.flush()
            if qb == NQB - 1:
                ref, row0 = self.on
                o = u2b(self.ot[64 * g:64 * g + 64, :]).T
                ref[row0:row0 + T // 2, 128 * g:128 * g + 128] = b2u(o)

        def main(self):
            NU = len(self.units)
            a, b = self.lag, self.eoff
            for i in range(NU):
                if i - a + b >= 0:
                    self.queue_exp(i - a + b)
                self.pvfrac = PVFRAC[self.br] if (i - a >= 0) else 0.0
                self.qk(i)
                for job in self.jobs.pop(i, []):
                    job()
                if i - a >= 0:
                    self.pv(i - a)
            self.pvfrac = 0.0
            return [((i - a + b) if (i - a + b) < NU else None, i - a) for i in range(NU, NU + a)]

    stB[XB0:XB0 + T // 2, :] = b2u(xa[...])
    def proj_loop(n, width, x_ref, w_ref, col_of, dma, epilogue):
        def body(j, c):
            dma(j)
            c0 = pl.multiple_of(col_of(j), 128)
            r = jnp.dot(x_ref[...], w_ref[:, pl.ds(c0, width)], preferred_element_type=f32)
            epilogue(j, r)
            return c
        lax.fori_loop(0, n, body, 0)

    def ep_q(q_ref, width):
        def f(j, r):
            q_ref[:, pl.ds(pl.multiple_of(j * width, 128), width)] = b2u((r * (SCALE * LOG2E)).astype(bf))
        return f

    def ep_k(st, width):
        def f(j, r):
            st[0:T // 2, pl.ds(pl.multiple_of(j * width, 128), width)] = b2u(r.astype(bf))
        return f

    def ep_v(vt, width):
        def f(j, r):
            vt[0, pl.ds(pl.multiple_of(j * (width // 2), 8), width // 2), :] = b2u(r.astype(bf).T)
        return f

    with scope("projB"):
        if first:
            nb = D // WB
            for t, ep in enumerate((ep_q(qb_, WB), ep_k(stB, WB), ep_v(vtb, WB))):
                proj_loop(nb, WB, xb, wb, lambda j, t=t: t * D + j * WB, lambda j, t=t: wait("B", t * nb + j), ep)
        else:
            x = xb[...]
            q = proj(x, wb, 0)
            qb_[...] = b2u((q * (SCALE * LOG2E)).astype(bf))
            store_k(stB, proj(x, wb, D))
            store_vt(vtb, proj(x, wb, 2 * D))
    attB = Att("B")
    with scope("attB"):
        restB = attB.main()
    with scope("projA"):
      if first:
        for eu, pu in restB:
            if eu is not None:
                attB.queue_exp(eu)
            fill.flush()
            attB.pv(pu)
        na = D // WA
        for t, (c, ep) in enumerate(((D, ep_k(ka, WA)), (0, ep_q(qa, WA)), (2 * D, ep_v(vta, WA)))):
            proj_loop(na, WA, xa, wa, lambda j, c=c: c + j * WA, lambda j, t=t: wait("A", t * na + j), ep)
      else:
        x = xa[...]
        nk = len(restB) + 1
        for i in range(nk):
            c0, c1 = 128 * ((8 * i) // nk), 128 * ((8 * (i + 1)) // nk)
            eu, pu = restB[i - 1] if i >= 1 else (None, None)
            if restB and i < len(restB) and restB[i][0] is not None and i >= KA0:
                pass
            if i >= 1 and eu is not None:
                attB.queue_exp(eu)
                lhs = anchored(stB, XB0, T // 16)
            else:
                lhs = x
            store_k(ka, proj(lhs, wa, D + c0, c1 - c0), c0)
            if pu is not None:
                attB.pv(pu)
        q = proj(x, wa, 0)
        qa[...] = b2u((q * (SCALE * LOG2E)).astype(bf))
        store_vt(vta, proj(x, wa, 2 * D))
    attA = Att("A")

    def outb_piece(c0, c1):
        def job():
            o = jnp.dot(u2b(stA[XB0:XB0 + T // 2, :]), wob[:, c0:c1], preferred_element_type=f32)
            out[:, D + c0:D + c1] = o.astype(bf)
        return job

    pieces = [outb_piece(PW * i, PW * i + PW) for i in range(D // PW)]
    wait("o", 0)
    ntail = LAG_A + 1
    nin = len(pieces) - min(ntail, PTAIL)
    for k in range(nin):
        attA.jobs.setdefault(PSTART + (k * (16 - PSTART)) // nin, []).append(pieces[k])
    with scope("attA"):
        restA = attA.main()
    with scope("outproj"):
        rest = pieces[nin:]
        for i in range(len(restA)):
            eu, pu = restA[i]
            if eu is not None:
                attA.queue_exp(eu)
            if i < len(rest):
                rest[i]()
            fill.flush()
            attA.pv(pu)
        for j in rest[len(restA):]:
            j()
        wait("o", 1)
        if first:
            def ep_o(j, r):
                out[:, pl.ds(pl.multiple_of(j * WA, 128), WA)] = r.astype(bf)
            def body(j, c):
                r = jnp.dot(u2b(ona[...]), woa[:, pl.ds(pl.multiple_of(j * WA, 128), WA)], preferred_element_type=f32)
                ep_o(j, r)
                return c
            lax.fori_loop(0, D // WA, body, 0)
        else:
            o = jnp.dot(u2b(ona[...]), woa[...], preferred_element_type=f32)
            out[:, 0:D] = o.astype(bf)


WB = 256
WA = 512
NB = 3 * D // WB
NA = 3 * D // WA
AHEAD = 2


def _kernel(zr, xa_h, xb_h, wa_h, wb_h, woa_h, wob_h, out_h,
            xa, xb, outb, wa, wb, woa, wob, qa, qb_, stA, stB, ka, pa, vta, vtb, ota, otb, ona, s0, s1, s2, biasb, biasa, biasm, biasa4, sems, xsem, osem):
    z = pl.multiple_of(zr[0], 8)
    z1 = zr[1]

    def cpB(c):
        c0 = pl.multiple_of(c * WB, 128) if not isinstance(c, int) else c * WB
        return pltpu.make_async_copy(wb_h.at[:, pl.ds(c0, WB)], wb.at[:, pl.ds(c0, WB)], sems.at[c])

    def cpA(c):
        na = D // WA
        if isinstance(c, int):
            c0 = (D, 0, 2 * D)[c // na] + (c % na) * WA
        else:
            t = c // na
            c0 = pl.multiple_of(jnp.where(t == 0, D, jnp.where(t == 1, 0, 2 * D)) + lax.rem(c, na) * WA, 128)
        return pltpu.make_async_copy(wa_h.at[:, pl.ds(c0, WA)], wa.at[:, pl.ds(c0, WA)], sems.at[NB + c])

    def cpO(c):
        return pltpu.make_async_copy((wob_h, woa_h)[c], (wob, woa)[c], sems.at[NB + NA + c])

    def issue(kind, c):
        if kind == "B":
            pl.when(c < NB)(lambda: cpB(c).start())
            pl.when(c >= NB)(lambda: cpA(c - NB).start())
        elif kind == "A":
            pl.when(c < NA)(lambda: cpA(c).start())
            pl.when(c == NA)(lambda: cpO(0).start())
            pl.when(c == NA + 1)(lambda: cpO(1).start())

    def wait_first(kind, c):
        if kind == "o":
            cpO(c).wait()
            return
        (cpB if kind == "B" else cpA)(c).wait()
        issue(kind, c + AHEAD)
        if kind == "A":
            @pl.when(c == NA - 1)
            def _():
                xcp(1, 1, 1).start()
                xcp(0, 1, 1).start()

    def xcp(which, step, slot):
        src, dst = ((xa_h, xa), (xb_h, xb))[which]
        return pltpu.make_async_copy(src.at[pl.ds(pl.multiple_of(step * T, T), T), :], dst.at[slot], xsem.at[2 * which + slot])

    def ocp(step, slot):
        return pltpu.make_async_copy(outb.at[slot], out_h.at[pl.ds(pl.multiple_of(step * T, T), T), :], osem.at[slot])

    def init_bias():
        jj = lax.broadcasted_iota(jnp.int32, (128, 128), 0)
        ii = lax.broadcasted_iota(jnp.int32, (128, 128), 1)
        biasb[0] = jnp.where(jj > ii, 0.0, NEG)
        biasb[1] = jnp.where(jj <= ii, 0.0, NEG)
        jj = lax.broadcasted_iota(jnp.int32, (144, 128), 0)
        ii = lax.broadcasted_iota(jnp.int32, (144, 128), 1)
        d = ii + 16 - jj
        biasa[...] = jnp.where((d >= 0) & (d < 16) & ((d & 1) == 0), 0.0, NEG)
        jj = lax.broadcasted_iota(jnp.int32, (64, 128), 0)
        ii = lax.broadcasted_iota(jnp.int32, (64, 128), 1)
        biasm[...] = jnp.where(jnp.where(ii < 64, jj - ii, ii - 63 - jj) > 0, 0.0, NEG)
        jj = lax.broadcasted_iota(jnp.int32, (48, 128), 0)
        ii = lax.broadcasted_iota(jnp.int32, (48, 128), 1)
        d = (ii & 31) + 16 - jj
        biasa4[...] = jnp.where((d >= 0) & (d < 16) & ((d & 1) == 0), 0.0, NEG)

    def run(first, step, slot, wait):
        _body(first, step, z, z1, xa.at[slot], xb.at[slot], wa, wb, woa, wob, outb.at[slot],
              qa, qb_, stA, stB, ka, pa, vta, vtb, ota, otb, ona, (s0, s1, s2), biasb, biasa, biasm, biasa4, wait)

    xcp(1, 0, 0).start()
    cpB(0).start()
    xcp(0, 0, 0).start()
    for c in range(1, AHEAD):
        cpB(c).start()
    init_bias()
    with scope("wait0"):
        xcp(1, 0, 0).wait()
        xcp(0, 0, 0).wait()

    run(True, 0, 0, wait_first)
    ocp(0, 0).start()

    def loop(step, carry):
        slot = lax.rem(step, 2)
        with scope("xwait"):
            xcp(1, step, slot).wait()
            xcp(0, step, slot).wait()

        @pl.when(step + 1 < NSTEP)
        def _():
            xcp(1, step + 1, 1 - slot).start()
            xcp(0, step + 1, 1 - slot).start()

        @pl.when(step >= 2)
        def _():
            ocp(step - 2, slot).wait()

        run(False, step, slot, lambda *a: None)
        ocp(step, slot).start()
        return carry

    lax.fori_loop(1, NSTEP, loop, 0)
    with scope("tail"):
        ocp(NSTEP - 2, NSTEP % 2).wait()
        ocp(NSTEP - 1, (NSTEP - 1) % 2).wait()


@jax.jit
def pallas_concat_heads__sliding_local_dilated__sliding_block__prompt_kernel(A_x, A_wqkv, A_wo, B_x, B_wqkv, B_wo):
    xa = A_x.reshape(S, D)
    xb = B_x.reshape(S, D)
    hbm = pl.BlockSpec(memory_space=pl.ANY)
    out = pl.pallas_call(
        _kernel,
        in_specs=[pl.BlockSpec(memory_space=pltpu.SMEM), hbm, hbm, hbm, hbm, hbm, hbm],
        out_specs=hbm,
        out_shape=jax.ShapeDtypeStruct((S, 2 * D), bf),
        scratch_shapes=[
            pltpu.VMEM((2, T, D), bf), pltpu.VMEM((2, T, D), bf), pltpu.VMEM((2, T, 2 * D), bf),
            pltpu.VMEM((D, 3 * D), bf), pltpu.VMEM((D, 3 * D), bf), pltpu.VMEM((D, D), bf), pltpu.VMEM((D, D), bf),
            pltpu.VMEM((T // 2, D), u32), pltpu.VMEM((T // 2, D), u32),
            pltpu.VMEM((STROWS, D), u32), pltpu.VMEM((STROWS, D), u32), pltpu.VMEM((KR, D), u32), pltpu.VMEM((224, D), u32),
            pltpu.VMEM((2, 512, T), u32), pltpu.VMEM((2, 512, T), u32),
            pltpu.VMEM((512, T), u32), pltpu.VMEM((512, T), u32), pltpu.VMEM((T // 2, D), u32),
            pltpu.VMEM((4, 384, 128), f32), pltpu.VMEM((4, 384, 128), f32), pltpu.VMEM((4, 384, 128), f32),
            pltpu.VMEM((2, 128, 128), f32), pltpu.VMEM((144, 128), f32), pltpu.VMEM((64, 128), f32), pltpu.VMEM((48, 128), f32),
            pltpu.SemaphoreType.DMA((NB + NA + 2,)), pltpu.SemaphoreType.DMA((4,)), pltpu.SemaphoreType.DMA((2,)),
        ],
        compiler_params=pltpu.CompilerParams(vmem_limit_bytes=100 * 1024 * 1024, flags=FLAGS),
        name="fused_attn",
    )(np.zeros((8,), np.int32), xa, xb, A_wqkv, B_wqkv, A_wo, B_wo)
    return out.reshape(1, S, 2 * D)
```

```python
import contextlib
import functools
import numpy as np
import jax
import jax.numpy as jnp
from jax import lax
from jax.experimental import pallas as pl
from jax.experimental.pallas import tpu as pltpu

S, D, H, DH = 2048, 1024, 32, 32
T = 256
NQB = T // 128
NSTEP = S // T
LOG2E = 1.4426950408889634
SCALE = DH ** -0.5
NEG = -1e30
bf = jnp.bfloat16
f32 = jnp.float32
u32 = jnp.uint32

NT = (((1,), (1,)), ((), ()))

LAG_B = 1
LAG_A = 2
SKIP_B = 1
SKIP_A = 0
END_B = 4
END_A = 0
SCOPES = 0
NOBC = 1
LATE1 = 1
OSPLIT = 1
UORD = 1
XALATE = 1
KP = 4
KH = [int(c) for c in str(1233)]
VSPLIT = 512
PW = 256
PSTART = 2
PTAIL = 2
MERGE_B = 1
EOFF_B = 0
EOFF_A = 0
PVFRAC = {"B": 0 / 100, "A": 0 / 100}
MERGE_A = 1
FLAGS = {}


def scope(n):
    on = SCOPES == 1 or (SCOPES >= 2 and n in ("wait0", "xwait", "tail"))
    return jax.named_scope(n) if on else contextlib.nullcontext()


b2u = lambda x: pltpu.bitcast(x, u32)
u2b = lambda x: pltpu.bitcast(x, bf)

KR = 2 * (T // 2)
PB0 = KR
LB0 = PB0 + 192
XB0 = LB0 + 32
STROWS = XB0 + T // 2


class Filler:
    def __init__(self):
        self.items = []

    def add(self, fn):
        self.items.append(fn)

    def flush(self, n=None):
        n = len(self.items) if n is None else min(n, len(self.items))
        for _ in range(n):
            self.items.pop(0)()

    def spread(self, nchunks, skip, end, keep=0):
        n = len(self.items) - keep
        act = max(1, nchunks - skip - end)
        done = 0
        res = []
        for j in range(nchunks):
            due = 0 if j < skip else min(n, -(-(j - skip + 1) * n // act))
            res.append(due - done)
            done = due
        return res


def _body(first, step, z, z1, outb_done, xa, xb, wa, wb, woa, wob, out,
          qa, qb_, stA, stB, ka, pa, vta, vtb, ota, otb, ona, s_sc, biasb, biasa, biasm, biasa4, wait):
    def scope(n):
        on = SCOPES == 1 or (SCOPES == 3 and first)
        return jax.named_scope(n) if on else contextlib.nullcontext()

    if first:
        cur, prv = 0, None
        zk = z
        zkp = None
    else:
        cur = lax.rem(step, 2)
        prv = 1 - cur
        zk = pl.multiple_of(z + cur * (T // 2), 8)
        zkp = pl.multiple_of(z + prv * (T // 2), 8)
    lane32 = lax.broadcasted_iota(jnp.int32, (64, 128), 1)
    hmask = [(lane32 >= 32 * h) & (lane32 < 32 * h + 32) for h in range(4)]
    fill = Filler()

    def ds8(zz, off, n):
        if isinstance(zz, int):
            return slice(zz + off, zz + off + n)
        return pl.ds(pl.multiple_of(zz + off, 8), n)
    zero = jnp.uint32(0)

    def proj(xv, w_ref, c0, n=D):
        return jnp.dot(xv, w_ref[:, c0:c0 + n], preferred_element_type=f32)

    def store_k(st, k, c0=0):
        ku = b2u(k.astype(bf))
        n = k.shape[1]
        if first:
            st[0:T // 2, c0:c0 + n] = ku
        else:
            st[pl.ds(pl.multiple_of(cur * (T // 2), 8), T // 2), c0:c0 + n] = ku

    def store_vt(vt, v, c0=0):
        vT = b2u(v.astype(bf).T)
        vt[cur, c0 // 2:c0 // 2 + vT.shape[0], :] = vT

    def anchored(st, row0, nchunk):
        sp = fill.spread(nchunk, 0, 1)
        cs = []
        for j in range(nchunk):
            fill.flush(sp[j])
            cs.append(u2b(st[pl.ds(pl.multiple_of(z + row0 + 8 * j, 8), 8), :]))
        fill.flush()
        return jnp.concatenate(cs, axis=0)

    class Att:
        def __init__(self, br):
            self.br = br
            isB = br == "B"
            self.hist = 256 if isB else 16
            self.q = qb_ if isB else qa
            self.st = stB if isB else ka
            self.pst = stB if isB else pa
            self.pz = z if isB else 0
            self.p0 = PB0 if isB else 0
            self.l0 = LB0 if isB else 192
            self.jobs = {}
            self.vt = vtb if isB else vta
            self.ot = otb if isB else ota
            self.on = (stA, XB0) if isB else (ona, 0)
            self.lag = LAG_B if isB else LAG_A
            self.eoff = EOFF_B if isB else EOFF_A
            self.nsb = self.lag - self.eoff + 1
            self.pvfrac = 0.0
            self.skip = SKIP_B if isB else SKIP_A
            self.end = END_B if isB else END_A
            self.units = [(g, qb) for g in range(8) for qb in range(NQB)]
            if first and isB and UORD:
                self.units = [(g, qb) for qb in (1, 0) for g in range(8)]
            self.lastqb = self.units[-1][1]
            self.ms = {}
            self.ls = {}

        def nk(self, qb):
            if first:
                return min(self.hist, 128 * qb) + 128
            return self.hist + 128

        def kchunk(self, g, qb, j):
            nk = self.nk(qb)
            r = 128 * qb + 128 - nk + 16 * j
            if r < 0:
                base, rr = zkp, (r + T) // 2
            else:
                base, rr = zk, r // 2
            return self.st[pl.ds(pl.multiple_of(base + rr, 8), 8), 128 * g:128 * g + 128]

        def qtile(self, u):
            g, qb = self.units[u]
            return self.q[64 * qb:64 * qb + 64, 128 * g:128 * g + 128]

        def merged(self, u):
            g, qb = self.units[u]
            return self.nk(qb) == self.hist + 128 and (MERGE_B if self.br == "B" else MERGE_A)

        def kloads(self, u, early=()):
            g, qb = self.units[u]
            nch = self.nk(qb) // 16
            ks = [None] * nch
            for j in early:
                ks[j] = self.kchunk(g, qb, j)
            rest = [j for j in range(nch) if j not in early]
            keep = int(len(fill.items) * self.pvfrac)
            sp = fill.spread(len(rest), min(self.skip, len(rest) // 3), min(self.end, len(rest) // 4), keep)
            for i, j in enumerate(rest):
                fill.flush(sp[i])
                ks[j] = self.kchunk(g, qb, j)
            fill.flush(len(fill.items) - keep)
            return ks

        def put(self, sb, h, parts):
            m = None
            for r0, p in parts:
                mm = jnp.max(p, axis=0, keepdims=True)
                m = mm if m is None else jnp.maximum(m, mm)
                sb[h, r0:r0 + p.shape[0], :] = p
            return m

        def qk(self, u):
            if self.merged(u):
                return (self.qk_b2 if self.br == "B" else self.qk_a4)(u)
            g, qb = self.units[u]
            nk = self.nk(qb)
            qi = self.qtile(u)
            qw = jnp.concatenate([u2b(jnp.where(hmask[h], qi, zero)) for h in range(4)], axis=0)
            ks = self.kloads(u)
            st = lax.dot_general(u2b(jnp.concatenate(ks, axis=0)), qw, NT, preferred_element_type=f32)
            sb = s_sc[u % self.nsb]
            ms = []
            for h in range(4):
                s = st[:, 128 * h:128 * h + 128]
                parts = []
                if self.br == "B":
                    nt = nk // 128
                    for t in range(nt):
                        p = s[128 * t:128 * t + 128]
                        if t == nt - 1:
                            p = p + biasb[1]
                        elif t == 0 and nt == 3:
                            p = p + biasb[0]
                        parts.append((128 * t, p))
                else:
                    parts.append((0, s + biasa[144 - nk:144, :]))
                ms.append(self.put(sb, h, parts))
            self.ms[u] = ms

        def qk_b2(self, u):
            qi = self.qtile(u)
            qm = [jnp.where(hmask[h], qi, zero) for h in range(4)]
            qr = pltpu.roll(qi[32:64], 32, 1)
            qx = [jnp.concatenate([qm[h][0:32], jnp.where(hmask[(h + 1) % 4][0:32], qr, zero)], axis=0) for h in range(4)]
            ks = self.kloads(u, early=(20, 21, 22, 23, 0, 1, 2, 3))
            ka = jnp.concatenate(ks[0:4], axis=0)
            kb = pltpu.roll(jnp.concatenate(ks[20:24], axis=0), 32, 1)
            even = (lane32[0:32] & 32) == 0
            l1 = u2b(jnp.where(even, ka, kb))
            l2 = u2b(jnp.where(even, kb, ka))
            s1 = lax.dot_general(l1, u2b(jnp.concatenate([qx[0], qx[2]], axis=0)), NT, preferred_element_type=f32)
            s2 = lax.dot_general(l2, u2b(jnp.concatenate([qx[1], qx[3]], axis=0)), NT, preferred_element_type=f32)
            main = u2b(jnp.concatenate(ks[4:20], axis=0))
            st = lax.dot_general(main, u2b(jnp.concatenate(qm, axis=0)), NT, preferred_element_type=f32)
            sb = s_sc[u % self.nsb]
            ms = []
            for h in range(4):
                s = st[:, 128 * h:128 * h + 128]
                sm = (s1, s2)[h % 2][:, 128 * (h // 2):128 * (h // 2) + 128]
                parts = [(0, sm + biasm[...]), (64, s[0:64] + biasb[0, 64:128, :]), (128, s[64:192]),
                         (256, s[192:256] + biasb[1, 0:64, :])]
                ms.append(self.put(sb, h, parts))
            self.ms[u] = ms

        def qk_a4(self, u):
            qi = self.qtile(u)
            qr = [qi[0:16]] + [pltpu.roll(qi[16 * m:16 * m + 16], 32 * m, 1) for m in (1, 2, 3)]
            ks = self.kloads(u)
            kr = []
            for m in range(4):
                w = jnp.concatenate(ks[2 * m:2 * m + 3], axis=0)
                kr.append(w if m == 0 else pltpu.roll(w, 32 * m, 1))
            grp = lane32[0:24] >> 5
            sb = s_sc[u % self.nsb]
            ms = []
            for h in range(4):
                rel = (grp - h) & 3
                lhs = jnp.where(rel == 0, kr[0], jnp.where(rel == 1, kr[1], jnp.where(rel == 2, kr[2], kr[3])))
                w = jnp.concatenate([jnp.where(hmask[(h + m) % 4][0:16], qr[m], zero) for m in range(4)], axis=0)
                s = lax.dot_general(u2b(lhs), u2b(w), NT, preferred_element_type=f32)
                ms.append(self.put(sb, h, [(0, s + biasa4[...])]))
            self.ms[u] = ms

        def nexp(self, u):
            g, qb = self.units[u]
            if self.merged(u):
                return 20 if self.br == "B" else 3
            return self.nk(qb) // 16

        def queue_exp(self, u, heads=(0, 1, 2, 3)):
            nch = self.nexp(u)
            ls = self.ls.setdefault(u, [None] * 4)
            ms = self.ms[u]
            sb = s_sc[u % self.nsb]
            lane0 = 512 * (u % 2)

            def mk(h, r):
                def fn():
                    s = sb[h + z1, 16 * r:16 * r + 16, :]
                    p = jnp.exp2(s - ms[h])
                    acc = p[0:8] + p[8:16]
                    ls[h] = acc if ls[h] is None else ls[h] + acc
                    self.pst[ds8(self.pz, self.p0 + 8 * r, 8), lane0 + 128 * h:lane0 + 128 * h + 128] = b2u(p.astype(bf))
                    if (r % 8 == 7 or r == nch - 1) and self.br == "B":
                        self.pst[ds8(self.pz, self.l0 + 8 * h, 8), lane0 + 128 * h:lane0 + 128 * h + 128] = pltpu.bitcast(ls[h], u32)
                return fn
            for h in heads:
                for r in range(nch):
                    fill.add(mk(h, r))

        def pv(self, u, heads=(0, 1, 2, 3)):
            g, qb = self.units[u]
            nk = self.nk(qb)
            lane0 = 512 * (u % 2)
            nt = -(-nk // 128)
            mg = self.merged(u)
            for h in heads:
                r0 = 64 * g + 16 * h
                tiles = []
                for t in range(nt):
                    kt = qb - (nt - 1 - t)
                    if kt < 0:
                        tiles.append(self.vt[prv, r0:r0 + 16, 128 * (kt + NQB):128 * (kt + NQB) + 128])
                    elif first:
                        tiles.append(self.vt[0, r0:r0 + 16, 128 * kt:128 * kt + 128])
                    else:
                        tiles.append(self.vt[cur, r0:r0 + 16, 128 * kt:128 * kt + 128])
                vt = u2b(jnp.concatenate(tiles, axis=1))
                n = self.nexp(u) * 8
                fill.flush(-(-len(fill.items) // (4 - h)) if h else len(fill.items) // 5)
                p = self.pst[ds8(self.pz, self.p0, n), lane0 + 128 * h:lane0 + 128 * h + 128]
                if mg and self.br == "B":
                    lo = lane32[0:32] < 64
                    p = jnp.concatenate([jnp.where(lo, p[0:32], zero), p[32:160], jnp.where(lo, zero, p[0:32])], axis=0)
                elif mg:
                    gm = [hmask[m][0:8] for m in range(4)]
                    p0, p1, p2 = p[0:8], p[8:16], p[16:24]
                    lo2 = [lane32[0:8] < 32 * (m + 1) for m in range(4)]
                    rows = [jnp.where(gm[0], p0, zero), jnp.where(gm[0], p1, zero)]
                    for m in range(3):
                        rows.append(jnp.where(gm[m], p2, jnp.where(gm[m + 1], p0, zero)))
                        rows.append(jnp.where(gm[m + 1], p1, zero))
                    rows.append(jnp.where(gm[3], p2, zero))
                    p = jnp.concatenate(rows, axis=0)
                if nk % 128:
                    p = jnp.concatenate([jnp.zeros(((128 * nt - nk) // 2, 128), u32), p], axis=0)
                ot = jnp.dot(vt, u2b(p), preferred_element_type=f32)
                l = jnp.sum(self.ls[u][h], axis=0, keepdims=True)
                self.ot[r0:r0 + 16, 128 * qb:128 * qb + 128] = b2u((ot * (1.0 / l)).astype(bf))
            fill.flush()
            if qb == self.lastqb and 3 in heads:
                ref, row0 = self.on
                o = u2b(self.ot[64 * g:64 * g + 64, :]).T
                ref[row0:row0 + T // 2, 128 * g:128 * g + 128] = b2u(o)

        def main(self):
            NU = len(self.units)
            a, b = self.lag, self.eoff
            for i in range(NU):
                if i - a + b >= 0:
                    self.queue_exp(i - a + b)
                self.pvfrac = PVFRAC[self.br] if (i - a >= 0) else 0.0
                self.qk(i)
                for job in self.jobs.pop(i, []):
                    job()
                if i - a >= 0:
                    self.pv(i - a)
            self.pvfrac = 0.0
            return [((i - a + b) if (i - a + b) < NU else None, i - a) for i in range(NU, NU + a)]

    def proj_loop(n, width, x_ref, w_ref, col_of, dma, epilogue):
        def body(j, c):
            dma(j)
            c0 = pl.multiple_of(col_of(j), 128)
            r = jnp.dot(x_ref[...], w_ref[:, pl.ds(c0, width)], preferred_element_type=f32)
            epilogue(j, r)
            return c
        lax.fori_loop(0, n, body, 0)

    def ep_q(q_ref, width):
        def f(j, r):
            q_ref[:, pl.ds(pl.multiple_of(j * width, 128), width)] = b2u((r * (SCALE * LOG2E)).astype(bf))
        return f

    def ep_k(st, width):
        def f(j, r):
            st[0:T // 2, pl.ds(pl.multiple_of(j * width, 128), width)] = b2u(r.astype(bf))
        return f

    def ep_v(vt, width):
        def f(j, r):
            vt[0, pl.ds(pl.multiple_of(j * (width // 2), 8), width // 2), :] = b2u(r.astype(bf).T)
        return f

    with scope("projB"):
        if first:
            nb = D // WB
            for t, ep in enumerate((ep_q(qb_, WB), ep_k(stB, WB), ep_v(vtb, WB))):
                proj_loop(nb, WB, xb, wb, lambda j, t=t: t * D + j * WB, lambda j, t=t: wait("B", t * nb + j), ep)
        else:
            x = xb[...]
            q = proj(x, wb, 0)
            qb_[...] = b2u((q * (SCALE * LOG2E)).astype(bf))
            store_k(stB, proj(x, wb, D))
            store_vt(vtb, proj(x, wb, 2 * D, VSPLIT), 0)
            vjob = lambda: store_vt(vtb, proj(x, wb, 2 * D + VSPLIT, D - VSPLIT), VSPLIT)
    attB = Att("B")
    if not first and VSPLIT < D:
        attB.jobs[0] = [vjob]
    with scope("attB"):
        restB = attB.main()
    with scope("projA"):
      if first:
        for eu, pu in restB:
            if eu is not None:
                attB.queue_exp(eu)
            fill.flush()
            attB.pv(pu)
        na = D // WA
        if XALATE:
            wait("x", 0)
        for t, (c, ep) in enumerate(((D, ep_k(ka, WA)), (0, ep_q(qa, WA)), (2 * D, ep_v(vta, WA)))):
            proj_loop(na, WA, xa, wa, lambda j, c=c: c + j * WA, lambda j, t=t: wait("A", t * na + j), ep)
      else:
        x = xa[...]
        (eu, pu), = restB
        assert eu == pu
        for i in range(KP):
            c0, c1 = 128 * ((8 * i) // KP), 128 * ((8 * (i + 1)) // KP)
            store_k(ka, proj(x, wa, D + c0, c1 - c0), c0)
            hs = [h for h in range(4) if KH[h] == i]
            if hs:
                attB.queue_exp(eu, hs)
                fill.flush()
                attB.pv(pu, hs)
        q = proj(x, wa, 0)
        qa[...] = b2u((q * (SCALE * LOG2E)).astype(bf))
        store_vt(vta, proj(x, wa, 2 * D))
    attA = Att("A")

    def outb_piece(c0, c1):
        def job():
            o = jnp.dot(u2b(stA[XB0:XB0 + T // 2, :]), wob[:, c0:c1], preferred_element_type=f32)
            out[:, D + c0:D + c1] = o.astype(bf)
        return job

    pieces = [outb_piece(PW * i, PW * i + PW) for i in range(D // PW)]
    wait("o", 0)
    ntail = LAG_A + 1
    nin = len(pieces) - min(ntail, PTAIL)
    for k in range(nin):
        attA.jobs.setdefault(PSTART + (k * (16 - PSTART)) // nin, []).append(pieces[k])
    with scope("attA"):
        restA = attA.main()
    with scope("outproj"):
        rest = pieces[nin:]
        for i in range(len(restA)):
            eu, pu = restA[i]
            if eu is not None:
                attA.queue_exp(eu)
            if i < len(rest):
                rest[i]()
            fill.flush()
            attA.pv(pu)
        for j in rest[len(restA):]:
            j()
        outb_done()
        wait("o", 1)
        if first:
            def ep_o(j, r):
                out[:, pl.ds(pl.multiple_of(j * WA, 128), WA)] = r.astype(bf)
            def body(j, c):
                r = jnp.dot(u2b(ona[...]), woa[:, pl.ds(pl.multiple_of(j * WA, 128), WA)], preferred_element_type=f32)
                ep_o(j, r)
                return c
            lax.fori_loop(0, D // WA, body, 0)
        else:
            o = jnp.dot(u2b(ona[...]), woa[...], preferred_element_type=f32)
            out[:, 0:D] = o.astype(bf)


WB = 512
WA = 512
NB = 3 * D // WB
NA = 3 * D // WA
AHEAD = 2


def _kernel(zr, xa_h, xb_h, wa_h, wb_h, woa_h, wob_h, out_h,
            xa, xb, outb, wa, wb, woa, wob, qa, qb_, stA, stB, ka, pa, vta, vtb, ota, otb, ona, s0, s1, s2, biasb, biasa, biasm, biasa4, sems, xsem, osem):
    z = pl.multiple_of(zr[0], 8)
    z1 = zr[1]

    def cpB(c):
        c0 = pl.multiple_of(c * WB, 128) if not isinstance(c, int) else c * WB
        return pltpu.make_async_copy(wb_h.at[:, pl.ds(c0, WB)], wb.at[:, pl.ds(c0, WB)], sems.at[c])

    def cpA(c):
        na = D // WA
        if isinstance(c, int):
            c0 = (D, 0, 2 * D)[c // na] + (c % na) * WA
        else:
            t = c // na
            c0 = pl.multiple_of(jnp.where(t == 0, D, jnp.where(t == 1, 0, 2 * D)) + lax.rem(c, na) * WA, 128)
        return pltpu.make_async_copy(wa_h.at[:, pl.ds(c0, WA)], wa.at[:, pl.ds(c0, WA)], sems.at[NB + c])

    def cpO(c):
        return pltpu.make_async_copy((wob_h, woa_h)[c], (wob, woa)[c], sems.at[NB + NA + c])

    def issue(kind, c):
        if kind == "B":
            pl.when(c < NB)(lambda: cpB(c).start())
            pl.when(c >= NB)(lambda: cpA(c - NB).start())
        elif kind == "A":
            pl.when(c < NA)(lambda: cpA(c).start())
            pl.when(c == NA + AHEAD - 2)(lambda: cpO(0).start())
            pl.when(c == NA + AHEAD - 1)(lambda: cpO(1).start())

    def wait_first(kind, c):
        if kind == "o":
            cpO(c).wait()
            return
        if kind == "x":
            xcp(0, 0, 0).wait()
            return
        (cpB if kind == "B" else cpA)(c).wait()
        issue(kind, c + AHEAD)
        if kind == "B" and XALATE:
            pl.when(c == NB - AHEAD - 1)(lambda: xcp(0, 0, 0).start())
        if kind == "A":
            @pl.when(c == NA - 1)
            def _():
                xcp(1, 1, 1).start()
                xcp(0, 1, 1).start()

    def xcp(which, step, slot):
        src, dst = ((xa_h, xa), (xb_h, xb))[which]
        return pltpu.make_async_copy(src.at[pl.ds(pl.multiple_of(step * T, T), T), :], dst.at[slot], xsem.at[2 * which + slot])

    def ocp(step, slot, half=None):
        rows = pl.ds(pl.multiple_of(step * T, T), T)
        if half is None:
            return pltpu.make_async_copy(outb.at[slot], out_h.at[rows, :], osem.at[slot])
        cols = slice(half * D, half * D + D)
        return pltpu.make_async_copy(outb.at[slot, :, cols], out_h.at[rows, cols], osem.at[2 * half + slot])

    def owait(step, slot):
        for hf in ((0, 1) if OSPLIT else (None,)):
            ocp(step, slot, hf).wait()

    def init_bias():
        jj = lax.broadcasted_iota(jnp.int32, (128, 128), 0)
        ii = lax.broadcasted_iota(jnp.int32, (128, 128), 1)
        biasb[0] = jnp.where(jj > ii, 0.0, NEG)
        biasb[1] = jnp.where(jj <= ii, 0.0, NEG)
        jj = lax.broadcasted_iota(jnp.int32, (144, 128), 0)
        ii = lax.broadcasted_iota(jnp.int32, (144, 128), 1)
        d = ii + 16 - jj
        biasa[...] = jnp.where((d >= 0) & (d < 16) & ((d & 1) == 0), 0.0, NEG)
        jj = lax.broadcasted_iota(jnp.int32, (64, 128), 0)
        ii = lax.broadcasted_iota(jnp.int32, (64, 128), 1)
        biasm[...] = jnp.where(jnp.where(ii < 64, jj - ii, ii - 63 - jj) > 0, 0.0, NEG)
        jj = lax.broadcasted_iota(jnp.int32, (48, 128), 0)
        ii = lax.broadcasted_iota(jnp.int32, (48, 128), 1)
        d = (ii & 31) + 16 - jj
        biasa4[...] = jnp.where((d >= 0) & (d < 16) & ((d & 1) == 0), 0.0, NEG)

    def run(first, step, slot, wait):
        _body(first, step, z, z1, (lambda: ocp(step, slot, 1).start()) if OSPLIT else (lambda: None), xa.at[slot], xb.at[slot], wa, wb, woa, wob, outb.at[slot],
              qa, qb_, stA, stB, ka, pa, vta, vtb, ota, otb, ona, (s0, s1, s2), biasb, biasa, biasm, biasa4, wait)

    xcp(1, 0, 0).start()
    cpB(0).start()
    if not XALATE:
        xcp(0, 0, 0).start()
    if not LATE1:
        for c in range(1, AHEAD):
            cpB(c).start()
    init_bias()
    with scope("wait0"):
        xcp(1, 0, 0).wait()
        if LATE1:
            for c in range(1, AHEAD):
                cpB(c).start()
        if not XALATE:
            xcp(0, 0, 0).wait()

    run(True, 0, 0, wait_first)
    ocp(0, 0, 0 if OSPLIT else None).start()

    def loop(step, carry):
        slot = lax.rem(step, 2)
        with scope("xwait"):
            xcp(1, step, slot).wait()
            xcp(0, step, slot).wait()

        @pl.when(step + 1 < NSTEP)
        def _():
            xcp(1, step + 1, 1 - slot).start()
            xcp(0, step + 1, 1 - slot).start()

        @pl.when(step >= 2)
        def _():
            owait(step - 2, slot)

        run(False, step, slot, lambda *a: None)
        ocp(step, slot, 0 if OSPLIT else None).start()
        return carry

    lax.fori_loop(1, NSTEP, loop, 0)
    with scope("tail"):
        owait(NSTEP - 2, NSTEP % 2)
        owait(NSTEP - 1, (NSTEP - 1) % 2)


@jax.jit
def pallas_concat_heads__sliding_local_dilated__sliding_block__prompt_kernel(A_x, A_wqkv, A_wo, B_x, B_wqkv, B_wo):
    xa = A_x.reshape(S, D)
    xb = B_x.reshape(S, D)
    hbm = pl.BlockSpec(memory_space=pl.ANY)
    out = pl.pallas_call(
        _kernel,
        in_specs=[pl.BlockSpec(memory_space=pltpu.SMEM), hbm, hbm, hbm, hbm, hbm, hbm],
        out_specs=hbm,
        out_shape=jax.ShapeDtypeStruct((S, 2 * D), bf),
        scratch_shapes=[
            pltpu.VMEM((2, T, D), bf), pltpu.VMEM((2, T, D), bf), pltpu.VMEM((2, T, 2 * D), bf),
            pltpu.VMEM((D, 3 * D), bf), pltpu.VMEM((D, 3 * D), bf), pltpu.VMEM((D, D), bf), pltpu.VMEM((D, D), bf),
            pltpu.VMEM((T // 2, D), u32), pltpu.VMEM((T // 2, D), u32),
            pltpu.VMEM((STROWS, D), u32), pltpu.VMEM((STROWS, D), u32), pltpu.VMEM((KR, D), u32), pltpu.VMEM((224, D), u32),
            pltpu.VMEM((2, 512, T), u32), pltpu.VMEM((2, 512, T), u32),
            pltpu.VMEM((512, T), u32), pltpu.VMEM((512, T), u32), pltpu.VMEM((T // 2, D), u32),
            pltpu.VMEM((4, 384, 128), f32), pltpu.VMEM((4, 384, 128), f32), pltpu.VMEM((4, 384, 128), f32),
            pltpu.VMEM((2, 128, 128), f32), pltpu.VMEM((144, 128), f32), pltpu.VMEM((64, 128), f32), pltpu.VMEM((48, 128), f32),
            pltpu.SemaphoreType.DMA((NB + NA + 2,)), pltpu.SemaphoreType.DMA((4,)), pltpu.SemaphoreType.DMA((4,)),
        ],
        compiler_params=pltpu.CompilerParams(vmem_limit_bytes=100 * 1024 * 1024, flags=FLAGS, disable_bounds_checks=bool(NOBC)),
        name="fused_attn",
    )(np.zeros((8,), np.int32), xa, xb, A_wqkv, B_wqkv, A_wo, B_wo)
    return out.reshape(1, S, 2 * D)
```

```python
import contextlib
import functools
import numpy as np
import jax
import jax.numpy as jnp
from jax import lax
from jax.experimental import pallas as pl
from jax.experimental.pallas import tpu as pltpu

S, D, H, DH = 2048, 1024, 32, 32
T = 256
NQB = T // 128
NSTEP = S // T
LOG2E = 1.4426950408889634
SCALE = DH ** -0.5
NEG = -1e30
bf = jnp.bfloat16
f32 = jnp.float32
u32 = jnp.uint32

NT = (((1,), (1,)), ((), ()))

LAG_B = 1
LAG_A = 3
SKIP_B = 1
SKIP_A = 0
END_B = 4
END_A = 0
SCOPES = 0
NOBC = 1
KFILL = 8
KF0 = 8
OUT32 = 0
oc = (lambda v: b2u(v)) if OUT32 else (lambda v: v)
LATE1 = 1
OSPLIT = 1
UORD = 1
XALATE = 1
KP = 4
KH = [int(c) for c in str(1233)]
VSPLIT = 512
PW = 128
PSTART = 2
PTAIL = 3
MERGE_B = 1
EOFF_B = 0
EOFF_A = 1
PVFRAC = {"B": 0 / 100, "A": 0 / 100}
MERGE_A = 1
FLAGS = {}


def scope(n):
    on = SCOPES == 1 or (SCOPES >= 2 and n in ("wait0", "xwait", "tail"))
    return jax.named_scope(n) if on else contextlib.nullcontext()


b2u = lambda x: pltpu.bitcast(x, u32)
u2b = lambda x: pltpu.bitcast(x, bf)

KR = 2 * (T // 2)
PB0 = KR
LB0 = PB0 + 192
XB0 = LB0 + 32
STROWS = XB0 + T // 2


class Filler:
    def __init__(self):
        self.items = []

    def add(self, fn):
        self.items.append(fn)

    def flush(self, n=None):
        n = len(self.items) if n is None else min(n, len(self.items))
        for _ in range(n):
            self.items.pop(0)()

    def spread(self, nchunks, skip, end, keep=0):
        n = len(self.items) - keep
        act = max(1, nchunks - skip - end)
        done = 0
        res = []
        for j in range(nchunks):
            due = 0 if j < skip else min(n, -(-(j - skip + 1) * n // act))
            res.append(due - done)
            done = due
        return res


def _body(first, step, z, z1, outb_done, xa, xb, wa, wb, woa, wob, out,
          qa, qb_, stA, stB, ka, pa, vta, vtb, ota, otb, ona, s_sc, biasb, biasa, biasm, biasa4, wait):
    def scope(n):
        on = SCOPES == 1 or (SCOPES == 3 and first)
        return jax.named_scope(n) if on else contextlib.nullcontext()

    if first:
        cur, prv = 0, None
        zk = z
        zkp = None
    else:
        cur = lax.rem(step, 2)
        prv = 1 - cur
        zk = pl.multiple_of(z + cur * (T // 2), 8)
        zkp = pl.multiple_of(z + prv * (T // 2), 8)
    lane32 = lax.broadcasted_iota(jnp.int32, (64, 128), 1)
    hmask = [(lane32 >= 32 * h) & (lane32 < 32 * h + 32) for h in range(4)]
    fill = Filler()

    def ds8(zz, off, n):
        if isinstance(zz, int):
            return slice(zz + off, zz + off + n)
        return pl.ds(pl.multiple_of(zz + off, 8), n)
    zero = jnp.uint32(0)

    def proj(xv, w_ref, c0, n=D):
        return jnp.dot(xv, u2b(w_ref[:, c0:c0 + n]), preferred_element_type=f32)

    def store_k(st, k, c0=0):
        ku = b2u(k.astype(bf))
        n = k.shape[1]
        if first:
            st[0:T // 2, c0:c0 + n] = ku
        else:
            st[pl.ds(pl.multiple_of(cur * (T // 2), 8), T // 2), c0:c0 + n] = ku

    def store_vt(vt, v, c0=0):
        vT = b2u(v.astype(bf).T)
        vt[cur, c0 // 2:c0 // 2 + vT.shape[0], :] = vT

    def anchored(st, row0, nchunk):
        sp = fill.spread(nchunk, 0, 1)
        cs = []
        for j in range(nchunk):
            fill.flush(sp[j])
            cs.append(u2b(st[pl.ds(pl.multiple_of(z + row0 + 8 * j, 8), 8), :]))
        fill.flush()
        return jnp.concatenate(cs, axis=0)

    class Att:
        def __init__(self, br):
            self.br = br
            isB = br == "B"
            self.hist = 256 if isB else 16
            self.q = qb_ if isB else qa
            self.st = stB if isB else ka
            self.pst = stB if isB else pa
            self.pz = z if isB else 0
            self.p0 = PB0 if isB else 0
            self.l0 = LB0 if isB else 192
            self.jobs = {}
            self.vt = vtb if isB else vta
            self.ot = otb if isB else ota
            self.on = (stA, XB0) if isB else (ona, 0)
            self.lag = LAG_B if isB else LAG_A
            self.eoff = EOFF_B if isB else EOFF_A
            self.nsb = self.lag - self.eoff + 1
            self.pvfrac = 0.0
            self.skip = SKIP_B if isB else SKIP_A
            self.end = END_B if isB else END_A
            self.units = [(g, qb) for g in range(8) for qb in range(NQB)]
            if first and isB and UORD:
                self.units = [(g, qb) for qb in (1, 0) for g in range(8)]
            self.lastqb = self.units[-1][1]
            self.ms = {}
            self.ls = {}

        def nk(self, qb):
            if first:
                return min(self.hist, 128 * qb) + 128
            return self.hist + 128

        def kchunk(self, g, qb, j):
            nk = self.nk(qb)
            r = 128 * qb + 128 - nk + 16 * j
            if r < 0:
                base, rr = zkp, (r + T) // 2
            else:
                base, rr = zk, r // 2
            return self.st[pl.ds(pl.multiple_of(base + rr, 8), 8), 128 * g:128 * g + 128]

        def qtile(self, u):
            g, qb = self.units[u]
            return self.q[64 * qb:64 * qb + 64, 128 * g:128 * g + 128]

        def merged(self, u):
            g, qb = self.units[u]
            return self.nk(qb) == self.hist + 128 and (MERGE_B if self.br == "B" else MERGE_A)

        def kloads(self, u, early=()):
            g, qb = self.units[u]
            nch = self.nk(qb) // 16
            ks = [None] * nch
            for j in early:
                ks[j] = self.kchunk(g, qb, j)
            rest = [j for j in range(nch) if j not in early]
            keep = int(len(fill.items) * self.pvfrac)
            sp = fill.spread(len(rest), min(self.skip, len(rest) // 3), min(self.end, len(rest) // 4), keep)
            for i, j in enumerate(rest):
                fill.flush(sp[i])
                ks[j] = self.kchunk(g, qb, j)
            fill.flush(len(fill.items) - keep)
            return ks

        def put(self, sb, h, parts):
            m = None
            for r0, p in parts:
                mm = jnp.max(p, axis=0, keepdims=True)
                m = mm if m is None else jnp.maximum(m, mm)
                sb[h, r0:r0 + p.shape[0], :] = p
            return m

        def qk(self, u):
            if self.merged(u):
                return (self.qk_b2 if self.br == "B" else self.qk_a4)(u)
            g, qb = self.units[u]
            nk = self.nk(qb)
            qi = self.qtile(u)
            qw = jnp.concatenate([u2b(jnp.where(hmask[h], qi, zero)) for h in range(4)], axis=0)
            ks = self.kloads(u)
            st = lax.dot_general(u2b(jnp.concatenate(ks, axis=0)), qw, NT, preferred_element_type=f32)
            sb = s_sc[u % self.nsb]
            ms = []
            for h in range(4):
                s = st[:, 128 * h:128 * h + 128]
                parts = []
                if self.br == "B":
                    nt = nk // 128
                    for t in range(nt):
                        p = s[128 * t:128 * t + 128]
                        if t == nt - 1:
                            p = p + biasb[1]
                        elif t == 0 and nt == 3:
                            p = p + biasb[0]
                        parts.append((128 * t, p))
                else:
                    parts.append((0, s + biasa[144 - nk:144, :]))
                ms.append(self.put(sb, h, parts))
            self.ms[u] = ms

        def qk_b2(self, u):
            qi = self.qtile(u)
            qm = [jnp.where(hmask[h], qi, zero) for h in range(4)]
            qr = pltpu.roll(qi[32:64], 32, 1)
            qx = [jnp.concatenate([qm[h][0:32], jnp.where(hmask[(h + 1) % 4][0:32], qr, zero)], axis=0) for h in range(4)]
            ks = self.kloads(u, early=(20, 21, 22, 23, 0, 1, 2, 3))
            ka = jnp.concatenate(ks[0:4], axis=0)
            kb = pltpu.roll(jnp.concatenate(ks[20:24], axis=0), 32, 1)
            even = (lane32[0:32] & 32) == 0
            l1 = u2b(jnp.where(even, ka, kb))
            l2 = u2b(jnp.where(even, kb, ka))
            s1 = lax.dot_general(l1, u2b(jnp.concatenate([qx[0], qx[2]], axis=0)), NT, preferred_element_type=f32)
            s2 = lax.dot_general(l2, u2b(jnp.concatenate([qx[1], qx[3]], axis=0)), NT, preferred_element_type=f32)
            main = u2b(jnp.concatenate(ks[4:20], axis=0))
            st = lax.dot_general(main, u2b(jnp.concatenate(qm, axis=0)), NT, preferred_element_type=f32)
            sb = s_sc[u % self.nsb]
            ms = []
            for h in range(4):
                s = st[:, 128 * h:128 * h + 128]
                sm = (s1, s2)[h % 2][:, 128 * (h // 2):128 * (h // 2) + 128]
                parts = [(0, sm + biasm[...]), (64, s[0:64] + biasb[0, 64:128, :]), (128, s[64:192]),
                         (256, s[192:256] + biasb[1, 0:64, :])]
                ms.append(self.put(sb, h, parts))
            self.ms[u] = ms

        def qk_a4(self, u):
            qi = self.qtile(u)
            qr = [qi[0:16]] + [pltpu.roll(qi[16 * m:16 * m + 16], 32 * m, 1) for m in (1, 2, 3)]
            ks = self.kloads(u)
            kr = []
            for m in range(4):
                w = jnp.concatenate(ks[2 * m:2 * m + 3], axis=0)
                kr.append(w if m == 0 else pltpu.roll(w, 32 * m, 1))
            grp = lane32[0:24] >> 5
            sb = s_sc[u % self.nsb]
            ms = []
            for h in range(4):
                rel = (grp - h) & 3
                lhs = jnp.where(rel == 0, kr[0], jnp.where(rel == 1, kr[1], jnp.where(rel == 2, kr[2], kr[3])))
                w = jnp.concatenate([jnp.where(hmask[(h + m) % 4][0:16], qr[m], zero) for m in range(4)], axis=0)
                s = lax.dot_general(u2b(lhs), u2b(w), NT, preferred_element_type=f32)
                ms.append(self.put(sb, h, [(0, s + biasa4[...])]))
            self.ms[u] = ms

        def nexp(self, u):
            g, qb = self.units[u]
            if self.merged(u):
                return 20 if self.br == "B" else 3
            return self.nk(qb) // 16

        def queue_exp(self, u, heads=(0, 1, 2, 3)):
            nch = self.nexp(u)
            ls = self.ls.setdefault(u, [None] * 4)
            ms = self.ms[u]
            sb = s_sc[u % self.nsb]
            lane0 = 512 * (u % 2)

            def mk(h, r):
                def fn():
                    s = sb[h + z1, 16 * r:16 * r + 16, :]
                    p = jnp.exp2(s - ms[h])
                    acc = p[0:8] + p[8:16]
                    ls[h] = acc if ls[h] is None else ls[h] + acc
                    self.pst[ds8(self.pz, self.p0 + 8 * r, 8), lane0 + 128 * h:lane0 + 128 * h + 128] = b2u(p.astype(bf))
                    if (r % 8 == 7 or r == nch - 1) and self.br == "B":
                        self.pst[ds8(self.pz, self.l0 + 8 * h, 8), lane0 + 128 * h:lane0 + 128 * h + 128] = pltpu.bitcast(ls[h], u32)
                return fn
            for h in heads:
                for r in range(nch):
                    fill.add(mk(h, r))

        def pv(self, u, heads=(0, 1, 2, 3)):
            g, qb = self.units[u]
            nk = self.nk(qb)
            lane0 = 512 * (u % 2)
            nt = -(-nk // 128)
            mg = self.merged(u)
            for h in heads:
                r0 = 64 * g + 16 * h
                tiles = []
                for t in range(nt):
                    kt = qb - (nt - 1 - t)
                    if kt < 0:
                        tiles.append(self.vt[prv, r0:r0 + 16, 128 * (kt + NQB):128 * (kt + NQB) + 128])
                    elif first:
                        tiles.append(self.vt[0, r0:r0 + 16, 128 * kt:128 * kt + 128])
                    else:
                        tiles.append(self.vt[cur, r0:r0 + 16, 128 * kt:128 * kt + 128])
                vt = u2b(jnp.concatenate(tiles, axis=1))
                n = self.nexp(u) * 8
                fill.flush(-(-len(fill.items) // (4 - h)) if h else len(fill.items) // 5)
                p = self.pst[ds8(self.pz, self.p0, n), lane0 + 128 * h:lane0 + 128 * h + 128]
                if mg and self.br == "B":
                    lo = lane32[0:32] < 64
                    p = jnp.concatenate([jnp.where(lo, p[0:32], zero), p[32:160], jnp.where(lo, zero, p[0:32])], axis=0)
                elif mg:
                    gm = [hmask[m][0:8] for m in range(4)]
                    p0, p1, p2 = p[0:8], p[8:16], p[16:24]
                    lo2 = [lane32[0:8] < 32 * (m + 1) for m in range(4)]
                    rows = [jnp.where(gm[0], p0, zero), jnp.where(gm[0], p1, zero)]
                    for m in range(3):
                        rows.append(jnp.where(gm[m], p2, jnp.where(gm[m + 1], p0, zero)))
                        rows.append(jnp.where(gm[m + 1], p1, zero))
                    rows.append(jnp.where(gm[3], p2, zero))
                    p = jnp.concatenate(rows, axis=0)
                if nk % 128:
                    p = jnp.concatenate([jnp.zeros(((128 * nt - nk) // 2, 128), u32), p], axis=0)
                ot = jnp.dot(vt, u2b(p), preferred_element_type=f32)
                l = jnp.sum(self.ls[u][h], axis=0, keepdims=True)
                self.ot[r0:r0 + 16, 128 * qb:128 * qb + 128] = b2u((ot * (1.0 / l)).astype(bf))
            fill.flush()
            if qb == self.lastqb and 3 in heads:
                ref, row0 = self.on
                o = u2b(self.ot[64 * g:64 * g + 64, :]).T
                ref[row0:row0 + T // 2, 128 * g:128 * g + 128] = b2u(o)

        def main(self):
            NU = len(self.units)
            a, b = self.lag, self.eoff
            for i in range(NU):
                if i - a + b >= 0:
                    self.queue_exp(i - a + b)
                self.pvfrac = PVFRAC[self.br] if (i - a >= 0) else 0.0
                self.qk(i)
                for job in self.jobs.pop(i, []):
                    job()
                if i - a >= 0:
                    self.pv(i - a)
            self.pvfrac = 0.0
            return [((i - a + b) if (i - a + b) < NU else None, i - a) for i in range(NU, NU + a)]

    def proj_loop(n, width, x_ref, w_ref, col_of, dma, epilogue):
        def body(j, c):
            dma(j)
            c0 = pl.multiple_of(col_of(j), 128)
            r = jnp.dot(u2b(x_ref[...]), u2b(w_ref[:, pl.ds(c0, width)]), preferred_element_type=f32)
            epilogue(j, r)
            return c
        lax.fori_loop(0, n, body, 0)

    def ep_q(q_ref, width):
        def f(j, r):
            q_ref[:, pl.ds(pl.multiple_of(j * width, 128), width)] = b2u((r * (SCALE * LOG2E)).astype(bf))
        return f

    def ep_k(st, width):
        def f(j, r):
            st[0:T // 2, pl.ds(pl.multiple_of(j * width, 128), width)] = b2u(r.astype(bf))
        return f

    def ep_v(vt, width):
        def f(j, r):
            vt[0, pl.ds(pl.multiple_of(j * (width // 2), 8), width // 2), :] = b2u(r.astype(bf).T)
        return f

    with scope("projB"):
        if first:
            nb = D // WB
            for t, ep in enumerate((ep_q(qb_, WB), ep_k(stB, WB), ep_v(vtb, WB))):
                proj_loop(nb, WB, xb, wb, lambda j, t=t: t * D + j * WB, lambda j, t=t: wait("B", t * nb + j), ep)
        else:
            x = u2b(xb[...])
            q = proj(x, wb, 0)
            qb_[...] = b2u((q * (SCALE * LOG2E)).astype(bf))
            store_k(stB, proj(x, wb, D))
            store_vt(vtb, proj(x, wb, 2 * D, VSPLIT), 0)
            vjob = lambda: store_vt(vtb, proj(x, wb, 2 * D + VSPLIT, D - VSPLIT), VSPLIT)
    attB = Att("B")
    if not first and VSPLIT < D:
        attB.jobs[0] = [vjob]
    if first and KFILL:
        def kpiece(i):
            def job():
                if i == 0:
                    wait("x", 0)
                if (i * D // KFILL) % WA == 0:
                    wait("A", (i * D // KFILL) // WA)
                w = D // KFILL
                store_k(ka, proj(u2b(xa[...]), wa, D + i * w, w), i * w)
            return job
        for i in range(KFILL):
            attB.jobs.setdefault(KF0 + (i * (16 - KF0)) // KFILL, []).append(kpiece(i))
    with scope("attB"):
        restB = attB.main()
    with scope("projA"):
      if first:
        for eu, pu in restB:
            if eu is not None:
                attB.queue_exp(eu)
            fill.flush()
            attB.pv(pu)
        na = D // WA
        if XALATE and not KFILL:
            wait("x", 0)
        for t, (c, ep) in enumerate(((D, ep_k(ka, WA)), (0, ep_q(qa, WA)), (2 * D, ep_v(vta, WA)))):
            if t == 0 and KFILL:
                continue
            proj_loop(na, WA, xa, wa, lambda j, c=c: c + j * WA, lambda j, t=t: wait("A", t * na + j), ep)
      else:
        x = u2b(xa[...])
        (eu, pu), = restB
        assert eu == pu
        for i in range(KP):
            c0, c1 = 128 * ((8 * i) // KP), 128 * ((8 * (i + 1)) // KP)
            store_k(ka, proj(x, wa, D + c0, c1 - c0), c0)
            hs = [h for h in range(4) if KH[h] == i]
            if hs:
                attB.queue_exp(eu, hs)
                fill.flush()
                attB.pv(pu, hs)
        q = proj(x, wa, 0)
        qa[...] = b2u((q * (SCALE * LOG2E)).astype(bf))
        store_vt(vta, proj(x, wa, 2 * D))
    attA = Att("A")

    def outb_piece(c0, c1):
        def job():
            o = jnp.dot(u2b(stA[XB0:XB0 + T // 2, :]), u2b(wob[:, c0:c1]), preferred_element_type=f32)
            out[:, D + c0:D + c1] = oc(o.astype(bf))
        return job

    pieces = [outb_piece(PW * i, PW * i + PW) for i in range(D // PW)]
    wait("o", 0)
    ntail = LAG_A + 1
    nin = len(pieces) - min(ntail, PTAIL)
    for k in range(nin):
        attA.jobs.setdefault(PSTART + (k * (16 - PSTART)) // nin, []).append(pieces[k])
    with scope("attA"):
        restA = attA.main()
    with scope("outproj"):
        rest = pieces[nin:]
        for i in range(len(restA)):
            eu, pu = restA[i]
            if eu is not None:
                attA.queue_exp(eu)
            if i < len(rest):
                rest[i]()
            fill.flush()
            attA.pv(pu)
        for j in rest[len(restA):]:
            j()
        outb_done()
        wait("o", 1)
        if first:
            def ep_o(j, r):
                out[:, pl.ds(pl.multiple_of(j * WA, 128), WA)] = oc(r.astype(bf))
            def body(j, c):
                r = jnp.dot(u2b(ona[...]), u2b(woa[:, pl.ds(pl.multiple_of(j * WA, 128), WA)]), preferred_element_type=f32)
                ep_o(j, r)
                return c
            lax.fori_loop(0, D // WA, body, 0)
        else:
            o = jnp.dot(u2b(ona[...]), u2b(woa[...]), preferred_element_type=f32)
            out[:, 0:D] = oc(o.astype(bf))


WB = 512
WA = 512
NB = 3 * D // WB
NA = 3 * D // WA
AHEAD = 2


def _kernel(zr, xa_h, xb_h, wa_h, wb_h, woa_h, wob_h, out_h,
            xa, xb, outb, wa, wb, woa, wob, qa, qb_, stA, stB, ka, pa, vta, vtb, ota, otb, ona, s0, s1, s2, biasb, biasa, biasm, biasa4, sems, xsem, osem):
    z = pl.multiple_of(zr[0], 8)
    z1 = zr[1]
    xa_h, xb_h, wa_h, wb_h, woa_h, wob_h = (r.bitcast(u32) for r in (xa_h, xb_h, wa_h, wb_h, woa_h, wob_h))
    out_h = out_h.bitcast(u32) if OUT32 else out_h

    def cpB(c):
        c0 = pl.multiple_of(c * WB, 128) if not isinstance(c, int) else c * WB
        return pltpu.make_async_copy(wb_h.at[:, pl.ds(c0, WB)], wb.at[:, pl.ds(c0, WB)], sems.at[c])

    def cpA(c):
        na = D // WA
        if isinstance(c, int):
            c0 = (D, 0, 2 * D)[c // na] + (c % na) * WA
        else:
            t = c // na
            c0 = pl.multiple_of(jnp.where(t == 0, D, jnp.where(t == 1, 0, 2 * D)) + lax.rem(c, na) * WA, 128)
        return pltpu.make_async_copy(wa_h.at[:, pl.ds(c0, WA)], wa.at[:, pl.ds(c0, WA)], sems.at[NB + c])

    def cpO(c):
        return pltpu.make_async_copy((wob_h, woa_h)[c], (wob, woa)[c], sems.at[NB + NA + c])

    def issue(kind, c):
        if kind == "B":
            pl.when(c < NB)(lambda: cpB(c).start())
            pl.when(c >= NB)(lambda: cpA(c - NB).start())
        elif kind == "A":
            pl.when(c < NA)(lambda: cpA(c).start())
            pl.when(c == NA + AHEAD - 2)(lambda: cpO(0).start())
            pl.when(c == NA + AHEAD - 1)(lambda: cpO(1).start())

    def wait_first(kind, c):
        if kind == "o":
            cpO(c).wait()
            return
        if kind == "x":
            xcp(0, 0, 0).wait()
            return
        (cpB if kind == "B" else cpA)(c).wait()
        issue(kind, c + AHEAD)
        if kind == "B" and XALATE:
            pl.when(c == NB - AHEAD - 1)(lambda: xcp(0, 0, 0).start())
        if kind == "A":
            @pl.when(c == NA - 1)
            def _():
                xcp(1, 1, 1).start()
                xcp(0, 1, 1).start()

    def xcp(which, step, slot):
        src, dst = ((xa_h, xa), (xb_h, xb))[which]
        return pltpu.make_async_copy(src.at[pl.ds(pl.multiple_of(step * (T // 2), T // 2), T // 2), :], dst.at[slot], xsem.at[2 * which + slot])

    def ocp(step, slot, half=None):
        rows = pl.ds(pl.multiple_of(step * (T // 2), T // 2), T // 2) if OUT32 else pl.ds(pl.multiple_of(step * T, T), T)
        if half is None:
            return pltpu.make_async_copy(outb.at[slot], out_h.at[rows, :], osem.at[slot])
        cols = slice(half * D, half * D + D)
        return pltpu.make_async_copy(outb.at[slot, :, cols], out_h.at[rows, cols], osem.at[2 * half + slot])

    def owait(step, slot):
        for hf in ((0, 1) if OSPLIT else (None,)):
            ocp(step, slot, hf).wait()

    def init_bias():
        jj = lax.broadcasted_iota(jnp.int32, (128, 128), 0)
        ii = lax.broadcasted_iota(jnp.int32, (128, 128), 1)
        biasb[0] = jnp.where(jj > ii, 0.0, NEG)
        biasb[1] = jnp.where(jj <= ii, 0.0, NEG)
        jj = lax.broadcasted_iota(jnp.int32, (144, 128), 0)
        ii = lax.broadcasted_iota(jnp.int32, (144, 128), 1)
        d = ii + 16 - jj
        biasa[...] = jnp.where((d >= 0) & (d < 16) & ((d & 1) == 0), 0.0, NEG)
        jj = lax.broadcasted_iota(jnp.int32, (64, 128), 0)
        ii = lax.broadcasted_iota(jnp.int32, (64, 128), 1)
        biasm[...] = jnp.where(jnp.where(ii < 64, jj - ii, ii - 63 - jj) > 0, 0.0, NEG)
        jj = lax.broadcasted_iota(jnp.int32, (48, 128), 0)
        ii = lax.broadcasted_iota(jnp.int32, (48, 128), 1)
        d = (ii & 31) + 16 - jj
        biasa4[...] = jnp.where((d >= 0) & (d < 16) & ((d & 1) == 0), 0.0, NEG)

    def run(first, step, slot, wait):
        _body(first, step, z, z1, (lambda: ocp(step, slot, 1).start()) if OSPLIT else (lambda: None), xa.at[slot], xb.at[slot], wa, wb, woa, wob, outb.at[slot],
              qa, qb_, stA, stB, ka, pa, vta, vtb, ota, otb, ona, (s0, s1, s2), biasb, biasa, biasm, biasa4, wait)

    xcp(1, 0, 0).start()
    cpB(0).start()
    if not XALATE:
        xcp(0, 0, 0).start()
    if not LATE1:
        for c in range(1, AHEAD):
            cpB(c).start()
    init_bias()
    with scope("wait0"):
        xcp(1, 0, 0).wait()
        if LATE1:
            for c in range(1, AHEAD):
                cpB(c).start()
        if not XALATE:
            xcp(0, 0, 0).wait()

    run(True, 0, 0, wait_first)
    ocp(0, 0, 0 if OSPLIT else None).start()

    def loop(step, carry):
        slot = lax.rem(step, 2)
        with scope("xwait"):
            xcp(1, step, slot).wait()
            xcp(0, step, slot).wait()

        @pl.when(step + 1 < NSTEP)
        def _():
            xcp(1, step + 1, 1 - slot).start()
            xcp(0, step + 1, 1 - slot).start()

        @pl.when(step >= 2)
        def _():
            owait(step - 2, slot)

        run(False, step, slot, lambda *a: None)
        ocp(step, slot, 0 if OSPLIT else None).start()
        return carry

    lax.fori_loop(1, NSTEP, loop, 0)
    with scope("tail"):
        owait(NSTEP - 2, NSTEP % 2)
        owait(NSTEP - 1, (NSTEP - 1) % 2)


@jax.jit
def pallas_concat_heads__sliding_local_dilated__sliding_block__prompt_kernel(A_x, A_wqkv, A_wo, B_x, B_wqkv, B_wo):
    xa = A_x.reshape(S, D)
    xb = B_x.reshape(S, D)
    hbm = pl.BlockSpec(memory_space=pl.ANY)
    out = pl.pallas_call(
        _kernel,
        in_specs=[pl.BlockSpec(memory_space=pltpu.SMEM), hbm, hbm, hbm, hbm, hbm, hbm],
        out_specs=hbm,
        out_shape=jax.ShapeDtypeStruct((S, 2 * D), bf),
        scratch_shapes=[
            pltpu.VMEM((2, T // 2, D), u32), pltpu.VMEM((2, T // 2, D), u32), pltpu.VMEM((2, T // 2, 2 * D), u32) if OUT32 else pltpu.VMEM((2, T, 2 * D), bf),
            pltpu.VMEM((D // 2, 3 * D), u32), pltpu.VMEM((D // 2, 3 * D), u32), pltpu.VMEM((D // 2, D), u32), pltpu.VMEM((D // 2, D), u32),
            pltpu.VMEM((T // 2, D), u32), pltpu.VMEM((T // 2, D), u32),
            pltpu.VMEM((STROWS, D), u32), pltpu.VMEM((STROWS, D), u32), pltpu.VMEM((KR, D), u32), pltpu.VMEM((224, D), u32),
            pltpu.VMEM((2, 512, T), u32), pltpu.VMEM((2, 512, T), u32),
            pltpu.VMEM((512, T), u32), pltpu.VMEM((512, T), u32), pltpu.VMEM((T // 2, D), u32),
            pltpu.VMEM((4, 384, 128), f32), pltpu.VMEM((4, 384, 128), f32), pltpu.VMEM((4, 384, 128), f32),
            pltpu.VMEM((2, 128, 128), f32), pltpu.VMEM((144, 128), f32), pltpu.VMEM((64, 128), f32), pltpu.VMEM((48, 128), f32),
            pltpu.SemaphoreType.DMA((NB + NA + 2,)), pltpu.SemaphoreType.DMA((4,)), pltpu.SemaphoreType.DMA((4,)),
        ],
        compiler_params=pltpu.CompilerParams(vmem_limit_bytes=100 * 1024 * 1024, flags=FLAGS, disable_bounds_checks=bool(NOBC)),
        name="fused_attn",
    )(np.zeros((8,), np.int32), xa, xb, A_wqkv, B_wqkv, A_wo, B_wo)
    return out.reshape(1, S, 2 * D)
```
